```python
import os as _os
_os.environ.setdefault("JAX_PLATFORMS", "cpu")
import jax
import jax.numpy as jnp

def _softmax(x, axis=-1):
    return jax.nn.softmax(x, axis=axis)
def _gelu(x):
    return jax.nn.gelu(x, approximate=True)
def _silu(x):
    return jax.nn.silu(x)
def _sigmoid(x):
    return jax.nn.sigmoid(x)
def _layernorm(x, axis=-1, eps=1e-5):
    m = jnp.mean(x, axis=axis, keepdims=True)
    v = jnp.var(x, axis=axis, keepdims=True)
    return (x - m) / jnp.sqrt(v + eps)
def _scatter_add(tgt, idx, src, axis=0):
    return tgt.at[idx].add(src)
def _segment_sum(src, seg, n):
    return jax.ops.segment_sum(src, seg, n)
class _Rng:
    def __init__(self, key):
        self._k = key
    def _next(self):
        self._k, sub = jax.random.split(self._k)
        return sub
    def normal(self, shape):
        return jax.random.normal(self._next(), shape, dtype=jnp.bfloat16)
    def randint(self, lo, hi, shape):
        return jax.random.randint(self._next(), shape, lo, hi, dtype=jnp.int32)
    def uniform(self, shape, lo=0.0, hi=1.0):
        return jax.random.uniform(self._next(), shape, jnp.bfloat16, lo, hi)
    def permutation(self, n):
        return jax.random.permutation(self._next(), n)


kernel_name = 'standalone__gqa_block_cached__sampling'

def setup_inputs():
    _rng = _Rng(jax.random.key(int.from_bytes(__import__("os").urandom(4), "little")))
    _w = (lambda a: (lambda t: t.astype(jnp.bfloat16) if jnp.issubdtype(t.dtype, jnp.floating) else t)(jnp.asarray(a)))
    B, Sq, D = 32, 16, 1024
    Hq, Hkv, Sk, Dh = 32, 4, 2048, 128
    assert Hq % Hkv == 0, (Hq, Hkv)
    return {
        "x": _w((lambda *s: _rng.normal(s) * 0.8)(B, Sq, D)),
        "k_cache": _w((lambda *s: _rng.normal(s) * 0.8)(B, Hkv, Sk, Dh)),
        "v_cache": _w((lambda *s: _rng.normal(s) * 0.05)(B, Hkv, Sk, Dh)),
        "wq": _w((lambda *s: _rng.normal(s) * 0.8)(D, Hq * Dh) * (D ** -0.5)),
        "wo": _w((lambda *s: _rng.normal(s) * 0.05)(Hq * Dh, D) * ((Hq * Dh) ** -0.5)),
    }

def reference(x, k_cache, v_cache, wq, wo):
    B, Sq, D = x.shape
    Hq, Dh = 32, 128
    Hkv = k_cache.shape[1]
    rep = Hq // Hkv
    q = (lambda x, *d: x.transpose(*d))((x @ wq).reshape(B, Sq, Hq, Dh), 0, 2, 1, 3)
    k = jnp.repeat(k_cache, rep, axis=1)
    v = jnp.repeat(v_cache, rep, axis=1)
    scores = jnp.einsum("bhqd,bhkd->bhqk", q, k) * (Dh ** -0.5)
    p = _softmax(scores, axis=-1)
    o = jnp.einsum("bhqk,bhkd->bhqd", p, v)
    return (lambda x, *d: x.transpose(*d))(o, 0, 2, 1, 3).reshape(B, Sq, Hq * Dh) @ wo
```

```python
import jax
import jax.numpy as jnp
from jax import lax
import jax.experimental.pallas as pl
import jax.experimental.pallas.tpu as pltpu

_LOG2E = 1.4426950408889634
_NK, _NV = 4, 8
_U = 2
_CB = 4


@jax.jit
def pallas_standalone__gqa_block_cached__sampling_kernel(
    x: jax.Array,
    k_cache: jax.Array,
    v_cache: jax.Array,
    wq: jax.Array,
    wo: jax.Array,
):
    B, SQ, D = x.shape
    _, HKV, SK, DH = k_cache.shape
    HQ = wq.shape[1] // DH
    REP = HQ // HKV
    M = B * SQ
    GW = REP * DH
    NT = B * HKV
    nk, nv, U, CB = _NK, _NV, _U, _CB
    NC = B // CB
    CR = CB * SQ

    def kern(x_hbm, k_hbm, v_hbm, wq_hbm, wo_hbm, out_hbm,
             x_v, wq_v, wo_v, q_scr, o_scr, acc, out_v, kbuf, vbuf,
             ksem, vsem, xsem, wqsem, wosem, osem):
        def k_copy(t):
            slot = t % nk
            return pltpu.make_async_copy(k_hbm.at[t % B, t // B], kbuf.at[slot], ksem.at[slot])

        def v_copy(t):
            slot = t % nv
            return pltpu.make_async_copy(v_hbm.at[t % B, t // B], vbuf.at[slot], vsem.at[slot])

        def wq_copy(h):
            return pltpu.make_async_copy(
                wq_hbm.at[:, pl.ds(pl.multiple_of(h * GW, GW), GW)], wq_v.at[h], wqsem.at[h])

        def wo_copy(h):
            return pltpu.make_async_copy(
                wo_hbm.at[pl.ds(pl.multiple_of(h * GW, GW), GW), :], wo_v.at[h], wosem.at[h])

        def out_copy(c):
            r = pl.ds(pl.multiple_of(c * CR, CR), CR)
            return pltpu.make_async_copy(out_v.at[r], out_hbm.at[r], osem.at[c])

        x_copy = pltpu.make_async_copy(x_hbm, x_v, xsem)

        @pl.loop(0, 1)
        def _(_):
            x_copy.start(priority=0)
            wq_copy(0).start(priority=0)

        @pl.loop(0, max(nk, nv))
        def _(t):
            @pl.when(t < nk)
            def _():
                k_copy(t).start(priority=0)

            @pl.when(t < nv)
            def _():
                v_copy(t).start(priority=1)

        acc[...] = jnp.zeros_like(acc)
        x_copy.wait()

        def attn_group(h, b0):
            ts = [h * B + b0 + u for u in range(U)]
            rs = [pl.multiple_of((b0 + u) * SQ, SQ) for u in range(U)]
            for t in ts:
                k_copy(t).wait()
            ss = []
            for t, r0 in zip(ts, rs):
                q = jnp.concatenate(
                    [q_scr[pl.ds(r0, SQ), j * DH:(j + 1) * DH] for j in range(REP)], axis=0)
                ss.append(lax.dot_general(q, kbuf[t % nk], (((1,), (1,)), ((), ())),
                                          preferred_element_type=jnp.float32))
            for t, r0, s in zip(ts, rs, ss):
                m = jnp.max(s, axis=-1, keepdims=True)
                p = jnp.exp2(s - m)
                l = jnp.sum(p, axis=-1, keepdims=True)
                p = p.astype(jnp.bfloat16)
                v_copy(t).wait()
                o = jnp.dot(p, vbuf[t % nv], preferred_element_type=jnp.float32)
                o = (o * (1.0 / l)).astype(jnp.bfloat16)
                for j in range(REP):
                    o_scr[pl.ds(r0, SQ), j * DH:(j + 1) * DH] = o[j * SQ:(j + 1) * SQ, :]
            for t in ts:
                @pl.when(t + nk < NT)
                def _():
                    k_copy(t + nk).start(priority=0)

                @pl.when(t + nv < NT)
                def _():
                    v_copy(t + nv).start(priority=1)

        def head_body(h, carry):
            wq_copy(h).wait()
            wo_copy(h).start(priority=0)

            @pl.when(h + 1 < HKV)
            def _():
                wq_copy(h + 1).start(priority=0)

            q = jnp.dot(x_v[...], wq_v[h], preferred_element_type=jnp.float32)
            q_scr[...] = (q * (DH ** -0.5 * _LOG2E)).astype(jnp.bfloat16)

            def chunk_body(c, carry2):
                def grp(g, cc):
                    attn_group(h, c * CB + g * U)
                    return cc
                lax.fori_loop(0, CB // U, grp, 0)
                r = pl.ds(pl.multiple_of(c * CR, CR), CR)

                @pl.when(c == 0)
                def _():
                    wo_copy(h).wait()

                acc[r, :] += jnp.dot(o_scr[r, :], wo_v[h], preferred_element_type=jnp.float32)

                @pl.when(h == HKV - 1)
                def _():
                    out_v[r, :] = acc[r, :].astype(jnp.bfloat16)
                    out_copy(c).start()
                return carry2
            lax.fori_loop(0, NC, chunk_body, 0)
            return carry
        lax.fori_loop(0, HKV, head_body, 0)
        for c in range(NC):
            out_copy(c).wait()

    anyspec = pl.BlockSpec(memory_space=pl.ANY)
    out = pl.pallas_call(
        kern,
        in_specs=[anyspec] * 5,
        out_specs=anyspec,
        out_shape=jax.ShapeDtypeStruct((M, D), jnp.bfloat16),
        scratch_shapes=[
            pltpu.VMEM((M, D), jnp.bfloat16),
            pltpu.VMEM((HKV, D, GW), jnp.bfloat16),
            pltpu.VMEM((HKV, GW, D), jnp.bfloat16),
            pltpu.VMEM((M, GW), jnp.bfloat16),
            pltpu.VMEM((M, GW), jnp.bfloat16),
            pltpu.VMEM((M, D), jnp.float32),
            pltpu.VMEM((M, D), jnp.bfloat16),
            pltpu.VMEM((nk, SK, DH), jnp.bfloat16),
            pltpu.VMEM((nv, SK, DH), jnp.bfloat16),
            pltpu.SemaphoreType.DMA((nk,)), pltpu.SemaphoreType.DMA((nv,)),
            pltpu.SemaphoreType.DMA(()), pltpu.SemaphoreType.DMA((HKV,)), pltpu.SemaphoreType.DMA((HKV,)),
            pltpu.SemaphoreType.DMA((NC,)),
        ],
        compiler_params=pltpu.CompilerParams(vmem_limit_bytes=120 * 1024 * 1024),
    )(x.reshape(M, D), k_cache, v_cache, wq, wo)
    return out.reshape(B, SQ, D)
```

```python
import jax
import jax.numpy as jnp
from jax import lax
import jax.experimental.pallas as pl
import jax.experimental.pallas.tpu as pltpu

_LOG2E = 1.4426950408889634


@jax.jit
def pallas_standalone__gqa_block_cached__sampling_kernel(
    x: jax.Array,
    k_cache: jax.Array,
    v_cache: jax.Array,
    wq: jax.Array,
    wo: jax.Array,
):
    B, SQ, D = x.shape
    _, HKV, SK, DH = k_cache.shape
    REP = wq.shape[1] // DH // HKV
    M = B * SQ
    GW = REP * DH
    NT = B * HKV
    scale = DH ** -0.5 * _LOG2E

    L = 4
    EARLY = 2
    SKIPS = (NT - B + 9, NT - B + 17)
    RK = RV = L + EARLY + 1
    CB = 4
    TD = 128
    WT = 16
    G = 4
    QCH = 4

    NC = B // CB
    NCT = NC * HKV
    CR = CB * SQ
    ND = SK // TD
    QR = M // QCH
    GK = SK // G
    TPG = GK // DH
    NWT = D // WT // QCH
    N0 = (HKV - 1) * B - 1

    def kern(x_hbm, k_hbm, v_hbm, wq_hbm, wo_hbm, out_hbm,
             x_v, wq_v, wo_v, q_scr, o_scr, acc, out_v, kv, s_a, s_b, m_a, m_b,
             ksem, vsem, xsem, wqsem, wosem, osem, osem2):

        def key_rows(j):
            return pl.ds(pl.multiple_of(j * TD, TD), TD)

        def k_tile(t, j):
            r = key_rows(j)
            return pltpu.make_async_copy(
                k_hbm.at[t % B, t // B, r], kv.at[t % RK, r], ksem.at[t % RK])

        def v_tile(t, j):
            r = key_rows(j)
            return pltpu.make_async_copy(
                v_hbm.at[t % B, t // B, r], kv.at[RK + t % RV, r], vsem.at[t % RV])

        def k_wait(t):
            s = t % RK
            pltpu.make_async_copy(kv.at[s], kv.at[s], ksem.at[s]).wait()

        def v_wait(t):
            s = t % RV
            pltpu.make_async_copy(kv.at[RK + s], kv.at[RK + s], vsem.at[s]).wait()

        def w_rows(i):
            return pl.ds(pl.multiple_of(i * WT, WT), WT)

        def wq_tile(g, i):
            return pltpu.make_async_copy(
                wq_hbm.at[w_rows(i), pl.ds(pl.multiple_of(g * GW, GW), GW)],
                wq_v.at[g, w_rows(i)], wqsem.at[g])

        def wo_tile(g, i):
            return pltpu.make_async_copy(
                wo_hbm.at[pl.ds(pl.multiple_of(g * GW + i * WT, WT), WT), :],
                wo_v.at[g, w_rows(i)], wosem.at[g])

        def x_tile(i):
            return pltpu.make_async_copy(x_hbm.at[w_rows(i)], x_v.at[w_rows(i)], xsem)

        def wq_wait(g):
            pltpu.make_async_copy(wq_v.at[g], wq_v.at[g], wqsem.at[g]).wait()

        def wo_wait(g):
            pltpu.make_async_copy(wo_v.at[g], wo_v.at[g], wosem.at[g]).wait()

        def out_bulk():
            r = pl.ds(0, M - CR)
            return pltpu.make_async_copy(out_v.at[r], out_hbm.at[r], osem2)

        def out_last():
            r = pl.ds(M - CR, CR)
            return pltpu.make_async_copy(out_v.at[r], out_hbm.at[r], osem)

        def qproj(g):
            @pl.loop(0, QCH)
            def _(i):
                r = pl.ds(pl.multiple_of(i * QR, QR), QR)
                q = jnp.dot(x_v[r, :], wq_v[g], preferred_element_type=jnp.float32)
                q_scr[g % 2, r, :] = (q * scale).astype(jnp.bfloat16)

                @pl.when(g + 1 < HKV)
                def _():
                    for k in range(NWT):
                        wq_tile(g + 1, i * NWT + k).start(priority=0)
                        wo_tile(g, i * NWT + k).start(priority=1)

                @pl.when(g + 1 >= HKV)
                def _():
                    per = EARLY * ND // QCH
                    for k in range(NWT):
                        wo_tile(g, i * NWT + k).start(priority=1)
                        for e in range(k * per // NWT, (k + 1) * per // NWT):
                            idx = i * per + e
                            t = N0 + L + idx // ND
                            k_tile(t, idx % ND).start(priority=0)
                            v_tile(t, idx % ND).start(priority=1)

        def load_q(t):
            r = pl.ds(pl.multiple_of((t % B) * SQ, SQ), SQ)
            return jnp.concatenate(
                [q_scr[(t // B) % 2, r, j * DH:(j + 1) * DH] for j in range(REP)], axis=0)

        def step(n, u, has_qk=True, has_refill=True, last=False):
            if u % 2 == 0:
                s_cur, m_cur, s_nxt, m_nxt = s_a, m_a, s_b, m_b
            else:
                s_cur, m_cur, s_nxt, m_nxt = s_b, m_b, s_a, m_a
            if has_qk:
                k_wait(n + 1)
            if not last:
                v_wait(n)
            if has_qk:
                q = load_q(n + 1)
            st = dict(mx=None, lsum=None, o=None, ps={})

            def do_qk(g):
                sg = lax.dot_general(
                    q, kv[(n + 1) % RK, pl.ds(g * GK, GK), :], (((1,), (1,)), ((), ())),
                    preferred_element_type=jnp.float32)
                s_nxt[:, g * GK:(g + 1) * GK] = sg
                for j in range(TPG):
                    sj = sg[:, j * DH:(j + 1) * DH]
                    st["mx"] = sj if st["mx"] is None else jnp.maximum(st["mx"], sj)

            def do_exp(g):
                m = m_cur[...]
                pj = []
                for j in range(TPG):
                    c0 = g * GK + j * DH
                    p = jnp.exp2(s_cur[:, c0:c0 + DH] - m)
                    st["lsum"] = p if st["lsum"] is None else st["lsum"] + p
                    pj.append(p.astype(jnp.bfloat16))
                st["ps"][g] = jnp.concatenate(pj, axis=1)

            def do_pv(g):
                og = jnp.dot(st["ps"][g], kv[RK + n % RV, pl.ds(g * GK, GK), :],
                             preferred_element_type=jnp.float32)
                st["o"] = og if st["o"] is None else st["o"] + og

            def do_refill():
                e = jnp.where(n >= N0, EARLY, 0)
                cond = None
                for sk in SKIPS:
                    e = e - jnp.where(n > sk, 1, 0)
                    if (sk - u) % CB == 0:
                        cond = (n != sk) if cond is None else cond & (n != sk)
                t = n + L + e
                for j in range(ND):
                    if cond is None:
                        k_tile(t, j).start(priority=0)
                        v_tile(t, j).start(priority=1)
                    else:
                        @pl.when(cond)
                        def _():
                            k_tile(t, j).start(priority=0)

                        @pl.when(cond)
                        def _():
                            v_tile(t, j).start(priority=1)

            if last:
                for g in range(G):
                    do_exp(g)
                v_wait(n)
                out_bulk().start()
                for g in range(G):
                    do_pv(g)
            else:
                for g in range(G + 1):
                    if g < G:
                        if has_qk:
                            do_qk(g)
                        do_exp(g)
                    if g >= 1:
                        do_pv(g - 1)
                    if has_refill and g == G - 1:
                        do_refill()
            if has_qk:
                m_nxt[...] = jnp.broadcast_to(
                    jnp.max(st["mx"], axis=-1, keepdims=True), (REP * SQ, DH))
            r = pl.ds(pl.multiple_of((n % B) * SQ, SQ), SQ)
            l = jnp.sum(st["lsum"], axis=-1, keepdims=True)
            o = (st["o"] * (1.0 / l)).astype(jnp.bfloat16)
            for j in range(REP):
                o_scr[r, j * DH:(j + 1) * DH] = o[j * SQ:(j + 1) * SQ, :]

        def oproj(c, h, final):
            r = pl.ds(pl.multiple_of((c % NC) * CR, CR), CR)
            y = jnp.dot(o_scr[r, :], wo_v[h], preferred_element_type=jnp.float32)
            if final:
                out_v[r, :] = (acc[r, :] + y).astype(jnp.bfloat16)
            else:
                acc[r, :] += y

        @pl.loop(0, M // WT // 2)
        def _(i):
            wq_tile(0, 4 * i).start(priority=0)
            x_tile(2 * i).start(priority=1)
            wq_tile(0, 4 * i + 1).start(priority=0)
            wq_tile(0, 4 * i + 2).start(priority=1)
            wq_tile(0, 4 * i + 3).start(priority=0)
            x_tile(2 * i + 1).start(priority=1)

        @pl.loop(0, L * ND)
        def _(i):
            k_tile(i // ND, i % ND).start(priority=0)
            v_tile(i // ND, i % ND).start(priority=1)

        acc[...] = jnp.zeros_like(acc)
        pltpu.make_async_copy(x_v, x_v, xsem).wait()
        wq_wait(0)
        qproj(0)
        k_wait(0)
        s0 = lax.dot_general(load_q(0), kv[0], (((1,), (1,)), ((), ())),
                             preferred_element_type=jnp.float32)
        s_a[...] = s0
        m_a[...] = jnp.broadcast_to(jnp.max(s0, axis=-1, keepdims=True), (REP * SQ, DH))

        def body(c, carry):
            h = c // NC
            for u in range(CB):
                if u == CB - 1:
                    @pl.when(c % NC == NC - 1)
                    def _():
                        wq_wait(h + 1)
                        qproj(h + 1)
                step(c * CB + u, u)

            @pl.when(c % NC == 0)
            def _():
                wo_wait(h)

            @pl.when(h < HKV - 1)
            def _():
                oproj(c, h, False)

            @pl.when(h == HKV - 1)
            def _():
                oproj(c, h, True)
            return carry
        lax.fori_loop(0, NCT - 1, body, 0)

        for u in range(CB):
            n = (NCT - 1) * CB + u
            step(n, u, has_qk=n + 1 < NT, has_refill=False, last=n == NT - 1)
        oproj(NCT - 1, HKV - 1, True)
        out_last().start()
        out_bulk().wait()
        out_last().wait()

    anyspec = pl.BlockSpec(memory_space=pl.ANY)
    out = pl.pallas_call(
        kern,
        in_specs=[anyspec] * 5,
        out_specs=anyspec,
        out_shape=jax.ShapeDtypeStruct((M, D), jnp.bfloat16),
        scratch_shapes=[
            pltpu.VMEM((M, D), jnp.bfloat16),
            pltpu.VMEM((HKV, D, GW), jnp.bfloat16),
            pltpu.VMEM((HKV, GW, D), jnp.bfloat16),
            pltpu.VMEM((2, M, GW), jnp.bfloat16),
            pltpu.VMEM((M, GW), jnp.bfloat16),
            pltpu.VMEM((M, D), jnp.float32),
            pltpu.VMEM((M, D), jnp.bfloat16),
            pltpu.VMEM((RK + RV, SK, DH), jnp.bfloat16),
            pltpu.VMEM((REP * SQ, SK), jnp.float32),
            pltpu.VMEM((REP * SQ, SK), jnp.float32),
            pltpu.VMEM((REP * SQ, DH), jnp.float32),
            pltpu.VMEM((REP * SQ, DH), jnp.float32),
            pltpu.SemaphoreType.DMA((RK,)),
            pltpu.SemaphoreType.DMA((RV,)),
            pltpu.SemaphoreType.DMA(()),
            pltpu.SemaphoreType.DMA((HKV,)),
            pltpu.SemaphoreType.DMA((HKV,)),
            pltpu.SemaphoreType.DMA(()),
            pltpu.SemaphoreType.DMA(()),
        ],
        compiler_params=pltpu.CompilerParams(
            vmem_limit_bytes=100 * 1024 * 1024,
            disable_semaphore_checks=True,
            disable_bounds_checks=True,
        ),
    )(x.reshape(M, D), k_cache, v_cache, wq, wo)
    return out.reshape(B, SQ, D)
```

```python
import functools

import jax
import jax.numpy as jnp
from jax import lax
import jax.experimental.pallas as pl
import jax.experimental.pallas.tpu as pltpu

_LOG2E = 1.4426950408889634


def _ds(start, size):
    if isinstance(start, int):
        return pl.ds(start, size)
    return pl.ds(pl.multiple_of(start, size), size)


@jax.jit
def pallas_standalone__gqa_block_cached__sampling_kernel(
    x: jax.Array,
    k_cache: jax.Array,
    v_cache: jax.Array,
    wq: jax.Array,
    wo: jax.Array,
):
    B, SQ, D = x.shape
    _, HKV, SK, DH = k_cache.shape
    REP = wq.shape[1] // DH // HKV
    M = B * SQ
    GW = REP * DH
    NT = B * HKV
    scale = DH ** -0.5 * _LOG2E

    L = 4
    EARLY = 2
    SKIPS = (NT - B + 9, NT - B + 17)
    KOFS = 10
    RING = L + EARLY + 1
    CB = 4
    TD = 128
    WT = 16
    G = 8
    QCH = 4

    NC = B // CB
    NCT = NC * HKV
    CR = CB * SQ
    ND = SK // TD
    QR = M // QCH
    GK = SK // G
    TPG = GK // DH
    NWT = D // WT // QCH
    N0 = (HKV - 1) * B - 1
    assert L == CB and EARLY * ND == QCH * (ND // 2) and CB % 2 == 0 and KOFS < ND

    def kern(x_hbm, k_hbm, v_hbm, wq_hbm, wo_hbm, out_hbm,
             x_v, wq_v, wo_v, q_scr, o_scr, acc, out_v, kv, s_a, s_b, m_a, m_b,
             ksem, vsem, xsem, wqsem, wosem, osem, osem2):

        def k_tile(t, j):
            r = pl.ds(j * TD, TD)
            return pltpu.make_async_copy(
                k_hbm.at[t % B, t // B, r], kv.at[t % RING, r], ksem.at[t % RING])

        def v_tile(t, j):
            r = pl.ds(j * TD, TD)
            return pltpu.make_async_copy(
                v_hbm.at[t % B, t // B, r], kv.at[RING + t % RING, r], vsem.at[t % RING])

        def issue_pair(m, j):
            if j >= KOFS:
                k_tile(m, j - KOFS).start(priority=0)
            elif not (isinstance(m, int) and m == 0):
                k_tile(m - 1, j - KOFS + ND).start(priority=0)
            v_tile(m, j).start(priority=1)

        def k_wait(t):
            s = t % RING
            pltpu.make_async_copy(kv.at[s], kv.at[s], ksem.at[s]).wait()

        def v_wait(t):
            s = t % RING
            pltpu.make_async_copy(kv.at[RING + s], kv.at[RING + s], vsem.at[s]).wait()

        def wq_tile(g, i):
            r = _ds(i * WT, WT)
            return pltpu.make_async_copy(
                wq_hbm.at[r, _ds(g * GW, GW)], wq_v.at[g, r], wqsem.at[g])

        def wo_tile(g, i):
            return pltpu.make_async_copy(
                wo_hbm.at[_ds(g * GW + i * WT, WT), :], wo_v.at[g, _ds(i * WT, WT)],
                wosem.at[g])

        def x_tile(i):
            r = _ds(i * WT, WT)
            return pltpu.make_async_copy(x_hbm.at[r], x_v.at[r], xsem)

        def wq_wait(g):
            pltpu.make_async_copy(wq_v.at[g], wq_v.at[g], wqsem.at[g]).wait()

        def wo_wait(g):
            pltpu.make_async_copy(wo_v.at[g], wo_v.at[g], wosem.at[g]).wait()

        def out_bulk():
            r = pl.ds(0, M - CR)
            return pltpu.make_async_copy(out_v.at[r], out_hbm.at[r], osem2)

        def out_last():
            r = pl.ds(M - CR, CR)
            return pltpu.make_async_copy(out_v.at[r], out_hbm.at[r], osem)

        def qproj(g):
            @pl.loop(0, QCH)
            def _(i):
                r = _ds(i * QR, QR)
                q = jnp.dot(x_v[r, :], wq_v[g], preferred_element_type=jnp.float32)
                q_scr[g % 2, r, :] = (q * scale).astype(jnp.bfloat16)

                @pl.when(g + 1 < HKV)
                def _():
                    for k in range(NWT):
                        wq_tile(g + 1, i * NWT + k).start(priority=0)
                        wo_tile(g, i * NWT + k).start(priority=1)

                @pl.when(g + 1 >= HKV)
                def _():
                    m = N0 + L + i // 2
                    for k in range(NWT):
                        wo_tile(g, i * NWT + k).start(priority=1)
                        for e in range(k * (ND // 2) // NWT, (k + 1) * (ND // 2) // NWT):
                            @pl.when(i % 2 == 0)
                            def _():
                                issue_pair(m, e)

                            @pl.when(i % 2 == 1)
                            def _():
                                issue_pair(m, ND // 2 + e)

        def load_q(t):
            r = _ds((t % B) * SQ, SQ)
            return jnp.concatenate(
                [q_scr[(t // B) % 2, r, j * DH:(j + 1) * DH] for j in range(REP)], axis=0)

        def step(n, u, has_qk=True, refill="ring"):
            if u % 2 == 0:
                s_cur, m_cur, s_nxt, m_nxt = s_a, m_a, s_b, m_b
            else:
                s_cur, m_cur, s_nxt, m_nxt = s_b, m_b, s_a, m_a
            if has_qk:
                k_wait(n + 1)
            v_wait(n)
            if has_qk:
                q = load_q(n + 1)
            else:
                out_bulk().start()
            st = dict(mx=None, lsum=None, o=None, ps={})

            def do_qk(g):
                sg = lax.dot_general(
                    q, kv[(n + 1) % RING, pl.ds(g * GK, GK), :], (((1,), (1,)), ((), ())),
                    preferred_element_type=jnp.float32)
                s_nxt[:, g * GK:(g + 1) * GK] = sg
                for j in range(TPG):
                    sj = sg[:, j * DH:(j + 1) * DH]
                    st["mx"] = sj if st["mx"] is None else jnp.maximum(st["mx"], sj)

            def do_exp(g):
                m = m_cur[...]
                pj = []
                for j in range(TPG):
                    c0 = g * GK + j * DH
                    p = jnp.exp2(s_cur[:, c0:c0 + DH] - m)
                    st["lsum"] = p if st["lsum"] is None else st["lsum"] + p
                    pj.append(p.astype(jnp.bfloat16))
                st["ps"][g] = jnp.concatenate(pj, axis=1)

            def do_pv(g):
                og = jnp.dot(st["ps"][g], kv[RING + n % RING, pl.ds(g * GK, GK), :],
                             preferred_element_type=jnp.float32)
                st["o"] = og if st["o"] is None else st["o"] + og

            def do_refill():
                if refill == "ring":
                    e = jnp.where(n >= N0, EARLY, 0)
                    for sk in SKIPS:
                        e = e - jnp.where(n > sk, 1, 0)
                    for j in range(ND):
                        issue_pair(n + L + e, j)
                elif refill == "rest":
                    for j in range(ND - KOFS, ND):
                        k_tile(NT - 1, j).start(priority=0)

            lag = 1 if has_qk else 0
            for g in range(G + lag):
                if g < G:
                    if has_qk:
                        do_qk(g)
                    do_exp(g)
                if g >= lag:
                    do_pv(g - lag)
                if g == G - 1:
                    do_refill()
            if has_qk:
                m_nxt[...] = jnp.broadcast_to(
                    jnp.max(st["mx"], axis=-1, keepdims=True), (REP * SQ, DH))
            r = _ds((n % B) * SQ, SQ)
            l = jnp.sum(st["lsum"], axis=-1, keepdims=True)
            o = (st["o"] * (1.0 / l)).astype(jnp.bfloat16)
            for j in range(REP):
                o_scr[r, j * DH:(j + 1) * DH] = o[j * SQ:(j + 1) * SQ, :]

        def oproj(c, h, final):
            r = _ds((c % NC) * CR, CR)
            y = jnp.dot(o_scr[r, :], wo_v[h], preferred_element_type=jnp.float32)
            if final:
                out_v[r, :] = (acc[r, :] + y).astype(jnp.bfloat16)
            else:
                acc[r, :] += y

        @pl.loop(0, M // WT // 2)
        def _(i):
            wq_tile(0, 4 * i).start(priority=0)
            x_tile(2 * i).start(priority=1)
            wq_tile(0, 4 * i + 1).start(priority=0)
            wq_tile(0, 4 * i + 2).start(priority=1)
            wq_tile(0, 4 * i + 3).start(priority=0)
            x_tile(2 * i + 1).start(priority=1)

        for j in range(ND):
            issue_pair(0, j)

        @pl.loop(1, L)
        def _(m):
            for j in range(ND):
                issue_pair(m, j)

        acc[...] = jnp.zeros_like(acc)
        pltpu.make_async_copy(x_v, x_v, xsem).wait()
        wq_wait(0)
        qproj(0)
        k_wait(0)
        s0 = lax.dot_general(load_q(0), kv[0], (((1,), (1,)), ((), ())),
                             preferred_element_type=jnp.float32)
        s_a[...] = s0
        m_a[...] = jnp.broadcast_to(jnp.max(s0, axis=-1, keepdims=True), (REP * SQ, DH))

        def body(c, carry):
            h = c // NC
            for u in range(CB):
                n = c * CB + u
                if u == CB - 1:
                    @pl.when(c % NC == NC - 1)
                    def _():
                        wq_wait(h + 1)
                        qproj(h + 1)
                sk = [s for s in SKIPS if (s - u) % CB == 0]
                if sk:
                    is_skip = functools.reduce(jnp.logical_or, [n == s for s in sk])

                    @pl.when(is_skip)
                    def _():
                        step(n, u, refill=None)

                    @pl.when(jnp.logical_not(is_skip))
                    def _():
                        step(n, u)
                else:
                    step(n, u)

            @pl.when(c % NC == 0)
            def _():
                wo_wait(h)

            @pl.when(h < HKV - 1)
            def _():
                oproj(c, h, False)

            @pl.when(h == HKV - 1)
            def _():
                oproj(c, h, True)
            return carry
        lax.fori_loop(0, NCT - 1, body, 0)

        for u in range(CB):
            n = (NCT - 1) * CB + u
            step(n, u, has_qk=n + 1 < NT, refill="rest" if u == 0 else None)
        oproj(NCT - 1, HKV - 1, True)
        out_last().start()
        out_bulk().wait()
        out_last().wait()

    anyspec = pl.BlockSpec(memory_space=pl.ANY)
    out = pl.pallas_call(
        kern,
        in_specs=[anyspec] * 5,
        out_specs=anyspec,
        out_shape=jax.ShapeDtypeStruct((M, D), jnp.bfloat16),
        scratch_shapes=[
            pltpu.VMEM((M, D), jnp.bfloat16),
            pltpu.VMEM((HKV, D, GW), jnp.bfloat16),
            pltpu.VMEM((HKV, GW, D), jnp.bfloat16),
            pltpu.VMEM((2, M, GW), jnp.bfloat16),
            pltpu.VMEM((M, GW), jnp.bfloat16),
            pltpu.VMEM((M, D), jnp.float32),
            pltpu.VMEM((M, D), jnp.bfloat16),
            pltpu.VMEM((2 * RING, SK, DH), jnp.bfloat16),
            pltpu.VMEM((REP * SQ, SK), jnp.float32),
            pltpu.VMEM((REP * SQ, SK), jnp.float32),
            pltpu.VMEM((REP * SQ, DH), jnp.float32),
            pltpu.VMEM((REP * SQ, DH), jnp.float32),
            pltpu.SemaphoreType.DMA((RING,)),
            pltpu.SemaphoreType.DMA((RING,)),
            pltpu.SemaphoreType.DMA(()),
            pltpu.SemaphoreType.DMA((HKV,)),
            pltpu.SemaphoreType.DMA((HKV,)),
            pltpu.SemaphoreType.DMA(()),
            pltpu.SemaphoreType.DMA(()),
        ],
        compiler_params=pltpu.CompilerParams(
            vmem_limit_bytes=100 * 1024 * 1024,
            disable_semaphore_checks=True,
            disable_bounds_checks=True,
        ),
    )(x.reshape(M, D), k_cache, v_cache, wq, wo)
    return out.reshape(B, SQ, D)
```

```python
import functools

import jax
import jax.numpy as jnp
from jax import lax
import jax.experimental.pallas as pl
import jax.experimental.pallas.tpu as pltpu

_LOG2E = 1.4426950408889634


def _ds(start, size):
    if isinstance(start, int):
        return pl.ds(start, size)
    return pl.ds(pl.multiple_of(start, size), size)


@jax.jit
def pallas_standalone__gqa_block_cached__sampling_kernel(
    x: jax.Array,
    k_cache: jax.Array,
    v_cache: jax.Array,
    wq: jax.Array,
    wo: jax.Array,
):
    B, SQ, D = x.shape
    _, HKV, SK, DH = k_cache.shape
    REP = wq.shape[1] // DH // HKV
    M = B * SQ
    GW = REP * DH
    NT = B * HKV
    scale = DH ** -0.5 * _LOG2E

    L = 4
    EARLY = 2
    SKIPS = (NT - B + 9, NT - B + 17)
    KOFS = 10
    RING = L + EARLY + 1
    CB = 4
    TD = 128
    WT = 16
    G = 8
    QCH = 4

    NC = B // CB
    NCT = NC * HKV
    CR = CB * SQ
    ND = SK // TD
    QR = M // QCH
    GK = SK // G
    TPG = GK // DH
    NWT = D // WT // QCH
    N0 = (HKV - 1) * B - 1
    assert L == CB and EARLY * ND == QCH * (ND // 2) and CB % 2 == 0 and KOFS < ND

    def kern(x_hbm, k_hbm, v_hbm, wq_hbm, wo_hbm, out_hbm,
             x_v, wq_v, wo_v, q_scr, o_scr, acc, out_v, kv, s_a, s_b, m_a, m_b,
             ksem, vsem, xsem, wqsem, wosem, osem, osem2):

        def k_tile(t, j):
            r = pl.ds(j * TD, TD)
            return pltpu.make_async_copy(
                k_hbm.at[t % B, t // B, r], kv.at[t % RING, r], ksem.at[t % RING])

        def v_tile(t, j):
            r = pl.ds(j * TD, TD)
            return pltpu.make_async_copy(
                v_hbm.at[t % B, t // B, r], kv.at[RING + t % RING, r], vsem.at[t % RING])

        def issue_pair(m, j):
            if j >= KOFS:
                k_tile(m, j - KOFS).start(priority=0)
            elif not (isinstance(m, int) and m == 0):
                k_tile(m - 1, j - KOFS + ND).start(priority=0)
            v_tile(m, j).start(priority=1)

        def k_wait(t):
            s = t % RING
            pltpu.make_async_copy(kv.at[s], kv.at[s], ksem.at[s]).wait()

        def v_wait(t):
            s = t % RING
            pltpu.make_async_copy(kv.at[RING + s], kv.at[RING + s], vsem.at[s]).wait()

        def wq_tile(g, i):
            r = _ds(i * WT, WT)
            return pltpu.make_async_copy(
                wq_hbm.at[r, _ds(g * GW, GW)], wq_v.at[g, r], wqsem.at[g])

        def wo_tile(g, i):
            return pltpu.make_async_copy(
                wo_hbm.at[_ds(g * GW + i * WT, WT), :], wo_v.at[g, _ds(i * WT, WT)],
                wosem.at[g])

        def x_tile(i):
            r = _ds(i * WT, WT)
            return pltpu.make_async_copy(x_hbm.at[r], x_v.at[r], xsem)

        def wq_wait(g):
            pltpu.make_async_copy(wq_v.at[g], wq_v.at[g], wqsem.at[g]).wait()

        def wo_wait(g):
            pltpu.make_async_copy(wo_v.at[g], wo_v.at[g], wosem.at[g]).wait()

        def out_bulk():
            r = pl.ds(0, M - CR)
            return pltpu.make_async_copy(out_v.at[r], out_hbm.at[r], osem2)

        def out_last():
            r = pl.ds(M - CR, CR)
            return pltpu.make_async_copy(out_v.at[r], out_hbm.at[r], osem)

        def qproj(g):
            @pl.loop(0, QCH)
            def _(i):
                r = _ds(i * QR, QR)
                q = jnp.dot(x_v[r, :], wq_v[g], preferred_element_type=jnp.float32)
                q_scr[g % 2, r, :] = (q * scale).astype(jnp.bfloat16)

                @pl.when(g + 1 < HKV)
                def _():
                    for k in range(NWT):
                        wq_tile(g + 1, i * NWT + k).start(priority=0)
                        wo_tile(g, i * NWT + k).start(priority=1)

                @pl.when(g + 1 >= HKV)
                def _():
                    m = N0 + L + i // 2
                    for k in range(NWT):
                        wo_tile(g, i * NWT + k).start(priority=1)
                        for e in range(k * (ND // 2) // NWT, (k + 1) * (ND // 2) // NWT):
                            @pl.when(i % 2 == 0)
                            def _():
                                issue_pair(m, e)

                            @pl.when(i % 2 == 1)
                            def _():
                                issue_pair(m, ND // 2 + e)

        def load_q(t):
            r = _ds((t % B) * SQ, SQ)
            return jnp.concatenate(
                [q_scr[(t // B) % 2, r, j * DH:(j + 1) * DH] for j in range(REP)], axis=0)

        def scores(t, s_ref, m_ref):
            s = lax.dot_general(load_q(t), kv[t % RING], (((1,), (1,)), ((), ())),
                                preferred_element_type=jnp.float32)
            s_ref[...] = s
            m_ref[...] = jnp.broadcast_to(jnp.max(s, axis=-1, keepdims=True), (REP * SQ, DH))

        def exp_group(s_ref, m_ref, g, st):
            m = m_ref[...]
            pj = []
            for j in range(TPG):
                c0 = g * GK + j * DH
                p = jnp.exp2(s_ref[:, c0:c0 + DH] - m)
                st["lsum"] = p if st["lsum"] is None else st["lsum"] + p
                pj.append(p.astype(jnp.bfloat16))
            st["ps"][g] = jnp.concatenate(pj, axis=1)

        def pv_group(t, g, st):
            og = jnp.dot(st["ps"][g], kv[RING + t % RING, pl.ds(g * GK, GK), :],
                         preferred_element_type=jnp.float32)
            st["o"] = og if st["o"] is None else st["o"] + og

        def finish(t, st):
            r = _ds((t % B) * SQ, SQ)
            l = jnp.sum(st["lsum"], axis=-1, keepdims=True)
            o = (st["o"] * (1.0 / l)).astype(jnp.bfloat16)
            for j in range(REP):
                o_scr[r, j * DH:(j + 1) * DH] = o[j * SQ:(j + 1) * SQ, :]

        def softmax_pv(t, s_ref, m_ref):
            st = dict(lsum=None, o=None, ps={})
            for g in range(G):
                exp_group(s_ref, m_ref, g, st)
                pv_group(t, g, st)
            finish(t, st)

        def step(n, u, refill="ring"):
            if u % 2 == 0:
                s_cur, m_cur, s_nxt, m_nxt = s_a, m_a, s_b, m_b
            else:
                s_cur, m_cur, s_nxt, m_nxt = s_b, m_b, s_a, m_a
            k_wait(n + 1)
            v_wait(n)
            q = load_q(n + 1)
            st = dict(mx=None, lsum=None, o=None, ps={})

            def do_qk(g):
                sg = lax.dot_general(
                    q, kv[(n + 1) % RING, pl.ds(g * GK, GK), :], (((1,), (1,)), ((), ())),
                    preferred_element_type=jnp.float32)
                s_nxt[:, g * GK:(g + 1) * GK] = sg
                for j in range(TPG):
                    sj = sg[:, j * DH:(j + 1) * DH]
                    st["mx"] = sj if st["mx"] is None else jnp.maximum(st["mx"], sj)

            def do_refill():
                if refill == "ring":
                    e = jnp.where(n >= N0, EARLY, 0)
                    for sk in SKIPS:
                        e = e - jnp.where(n > sk, 1, 0)
                    for j in range(ND):
                        issue_pair(n + L + e, j)
                elif refill == "rest":
                    for j in range(ND - KOFS, ND):
                        k_tile(NT - 1, j).start(priority=0)

            for g in range(G + 1):
                if g < G:
                    do_qk(g)
                    exp_group(s_cur, m_cur, g, st)
                if g >= 1:
                    pv_group(n, g - 1, st)
                if g == G - 1:
                    do_refill()
            m_nxt[...] = jnp.broadcast_to(
                jnp.max(st["mx"], axis=-1, keepdims=True), (REP * SQ, DH))
            finish(n, st)

        def oproj(c, h, final):
            r = _ds((c % NC) * CR, CR)
            y = jnp.dot(o_scr[r, :], wo_v[h], preferred_element_type=jnp.float32)
            if final:
                out_v[r, :] = (acc[r, :] + y).astype(jnp.bfloat16)
            else:
                acc[r, :] += y

        @pl.loop(0, M // WT // 2)
        def _(i):
            wq_tile(0, 4 * i).start(priority=0)
            x_tile(2 * i).start(priority=1)
            wq_tile(0, 4 * i + 1).start(priority=0)
            wq_tile(0, 4 * i + 2).start(priority=1)
            wq_tile(0, 4 * i + 3).start(priority=0)
            x_tile(2 * i + 1).start(priority=1)

        for j in range(ND):
            issue_pair(0, j)

        @pl.loop(1, L)
        def _(m):
            for j in range(ND):
                issue_pair(m, j)

        acc[...] = jnp.zeros_like(acc)
        pltpu.make_async_copy(x_v, x_v, xsem).wait()
        wq_wait(0)
        qproj(0)
        k_wait(0)
        scores(0, s_a, m_a)

        def body(c, carry):
            h = c // NC
            for u in range(CB):
                n = c * CB + u
                if u == CB - 1:
                    @pl.when(c % NC == NC - 1)
                    def _():
                        wq_wait(h + 1)
                        qproj(h + 1)
                sk = [s for s in SKIPS if (s - u) % CB == 0]
                if sk:
                    is_skip = functools.reduce(jnp.logical_or, [n == s for s in sk])

                    @pl.when(is_skip)
                    def _():
                        step(n, u, refill=None)

                    @pl.when(jnp.logical_not(is_skip))
                    def _():
                        step(n, u)
                else:
                    step(n, u)

            @pl.when(c % NC == 0)
            def _():
                wo_wait(h)

            @pl.when(h < HKV - 1)
            def _():
                oproj(c, h, False)

            @pl.when(h == HKV - 1)
            def _():
                oproj(c, h, True)
            return carry
        lax.fori_loop(0, NCT - 1, body, 0)

        for u in range(CB - 2):
            step((NCT - 1) * CB + u, u, refill="rest" if u == 0 else None)
        n = NT - 2
        k_wait(n + 1)
        scores(n + 1, s_b, m_b)
        v_wait(n)
        softmax_pv(n, s_a, m_a)
        v_wait(n + 1)
        out_bulk().start()
        softmax_pv(n + 1, s_b, m_b)
        oproj(NCT - 1, HKV - 1, True)
        out_last().start()
        out_bulk().wait()
        out_last().wait()

    anyspec = pl.BlockSpec(memory_space=pl.ANY)
    out = pl.pallas_call(
        kern,
        in_specs=[anyspec] * 5,
        out_specs=anyspec,
        out_shape=jax.ShapeDtypeStruct((M, D), jnp.bfloat16),
        scratch_shapes=[
            pltpu.VMEM((M, D), jnp.bfloat16),
            pltpu.VMEM((HKV, D, GW), jnp.bfloat16),
            pltpu.VMEM((HKV, GW, D), jnp.bfloat16),
            pltpu.VMEM((2, M, GW), jnp.bfloat16),
            pltpu.VMEM((M, GW), jnp.bfloat16),
            pltpu.VMEM((M, D), jnp.float32),
            pltpu.VMEM((M, D), jnp.bfloat16),
            pltpu.VMEM((2 * RING, SK, DH), jnp.bfloat16),
            pltpu.VMEM((REP * SQ, SK), jnp.float32),
            pltpu.VMEM((REP * SQ, SK), jnp.float32),
            pltpu.VMEM((REP * SQ, DH), jnp.float32),
            pltpu.VMEM((REP * SQ, DH), jnp.float32),
            pltpu.SemaphoreType.DMA((RING,)),
            pltpu.SemaphoreType.DMA((RING,)),
            pltpu.SemaphoreType.DMA(()),
            pltpu.SemaphoreType.DMA((HKV,)),
            pltpu.SemaphoreType.DMA((HKV,)),
            pltpu.SemaphoreType.DMA(()),
            pltpu.SemaphoreType.DMA(()),
        ],
        compiler_params=pltpu.CompilerParams(
            vmem_limit_bytes=100 * 1024 * 1024,
            disable_semaphore_checks=True,
            disable_bounds_checks=True,
        ),
    )(x.reshape(M, D), k_cache, v_cache, wq, wo)
    return out.reshape(B, SQ, D)
```

```python
import jax
import jax.numpy as jnp
from jax import lax
import jax.experimental.pallas as pl
import jax.experimental.pallas.tpu as pltpu

_LOG2E = 1.4426950408889634


def _ds(start, size):
    if isinstance(start, int):
        return pl.ds(start, size)
    return pl.ds(pl.multiple_of(start, size), size)


@jax.jit
def pallas_standalone__gqa_block_cached__sampling_kernel(
    x: jax.Array,
    k_cache: jax.Array,
    v_cache: jax.Array,
    wq: jax.Array,
    wo: jax.Array,
):
    B, SQ, D = x.shape
    _, HKV, SK, DH = k_cache.shape
    W = wq.shape[1]
    GW = W // HKV
    REP = GW // DH
    M = B * SQ
    NT = B * HKV
    scale = DH ** -0.5 * _LOG2E

    L = 4
    KOFS = 10
    RING = L + 1
    CB = 4
    TD = 128
    G = 8
    QCH = 4
    WO_PRE = 48
    WO_STEP = 20

    NC = B // CB
    NCT = NC * HKV
    CR = CB * SQ
    ND = SK // TD
    GK = SK // G
    TPG = GK // DH
    QR = M // QCH
    XR = 16
    WQR, WQC = 8, W // 2
    WOR = 16
    NXP = M // XR // 2
    NQP = D // WQR
    NOP = W // WOR // 2
    assert L == CB and CB % 2 == 0 and KOFS < ND and WO_PRE + QCH * WO_STEP <= NOP

    def kern(x_hbm, k_hbm, v_hbm, wq_hbm, wo_hbm, out_hbm,
             x_v, wq_v, wo_v, q_scr, o_scr, acc, out_v, kv, s_a, s_b, m_a, m_b,
             ksem, vsem, xsem, wqsem, wosem, osem, osem2):

        def k_tile(t, j):
            r = pl.ds(j * TD, TD)
            return pltpu.make_async_copy(
                k_hbm.at[t % B, t // B, r], kv.at[t % RING, r], ksem.at[t % RING])

        def v_tile(t, j):
            r = pl.ds(j * TD, TD)
            return pltpu.make_async_copy(
                v_hbm.at[t % B, t // B, r], kv.at[RING + t % RING, r], vsem.at[t % RING])

        def kv_pair(m, j):
            if j >= KOFS:
                k_tile(m, j - KOFS).start(priority=0)
            elif not (isinstance(m, int) and m == 0):
                k_tile(m - 1, j - KOFS + ND).start(priority=0)
            v_tile(m, j).start(priority=1)

        def k_wait(t):
            s = t % RING
            pltpu.make_async_copy(kv.at[s], kv.at[s], ksem.at[s]).wait()

        def v_wait(t):
            s = t % RING
            pltpu.make_async_copy(kv.at[RING + s], kv.at[RING + s], vsem.at[s]).wait()

        def x_pair(i):
            for p in range(2):
                r = _ds((2 * i + p) * XR, XR)
                pltpu.make_async_copy(x_hbm.at[r], x_v.at[r], xsem).start(priority=p)

        def wq_pair(i):
            for p in range(2):
                t = i + p * NQP
                r, c = _ds((t // 2) * WQR, WQR), _ds((t % 2) * WQC, WQC)
                pltpu.make_async_copy(wq_hbm.at[r, c], wq_v.at[r, c], wqsem).start(priority=p)

        def wo_pair(i):
            for p in range(2):
                r = _ds((i + p * NOP) * WOR, WOR)
                pltpu.make_async_copy(wo_hbm.at[r], wo_v.at[r], wosem).start(priority=p)

        def out_bulk():
            r = pl.ds(0, M - CR)
            return pltpu.make_async_copy(out_v.at[r], out_hbm.at[r], osem2)

        def out_last():
            r = pl.ds(M - CR, CR)
            return pltpu.make_async_copy(out_v.at[r], out_hbm.at[r], osem)

        def qproj(g, r):
            q = jnp.dot(x_v[r, :], wq_v[:, _ds(g * GW, GW)], preferred_element_type=jnp.float32)
            q_scr[g % 2, r, :] = (q * scale).astype(jnp.bfloat16)

        def load_q(t):
            r = _ds((t % B) * SQ, SQ)
            return jnp.concatenate(
                [q_scr[(t // B) % 2, r, j * DH:(j + 1) * DH] for j in range(REP)], axis=0)

        def scores(t, s_ref, m_ref):
            s = lax.dot_general(load_q(t), kv[t % RING], (((1,), (1,)), ((), ())),
                                preferred_element_type=jnp.float32)
            s_ref[...] = s
            m_ref[...] = jnp.broadcast_to(jnp.max(s, axis=-1, keepdims=True), (REP * SQ, DH))

        def exp_group(s_ref, m_ref, g, st):
            m = m_ref[...]
            pj = []
            for j in range(TPG):
                c0 = g * GK + j * DH
                p = jnp.exp2(s_ref[:, c0:c0 + DH] - m)
                st["lsum"] = p if st["lsum"] is None else st["lsum"] + p
                pj.append(p.astype(jnp.bfloat16))
            st["ps"][g] = jnp.concatenate(pj, axis=1)

        def pv_group(t, g, st):
            og = jnp.dot(st["ps"][g], kv[RING + t % RING, pl.ds(g * GK, GK), :],
                         preferred_element_type=jnp.float32)
            st["o"] = og if st["o"] is None else st["o"] + og

        def finish(t, st):
            r = _ds((t % B) * SQ, SQ)
            l = jnp.sum(st["lsum"], axis=-1, keepdims=True)
            o = (st["o"] * (1.0 / l)).astype(jnp.bfloat16)
            for j in range(REP):
                o_scr[r, j * DH:(j + 1) * DH] = o[j * SQ:(j + 1) * SQ, :]

        def softmax_pv(t, s_ref, m_ref):
            st = dict(lsum=None, o=None, ps={})
            for g in range(G):
                exp_group(s_ref, m_ref, g, st)
                pv_group(t, g, st)
            finish(t, st)

        def step(n, u, refill):
            if u % 2 == 0:
                s_cur, m_cur, s_nxt, m_nxt = s_a, m_a, s_b, m_b
            else:
                s_cur, m_cur, s_nxt, m_nxt = s_b, m_b, s_a, m_a
            k_wait(n + 1)
            v_wait(n)
            q = load_q(n + 1)
            st = dict(mx=None, lsum=None, o=None, ps={})

            def do_qk(g):
                sg = lax.dot_general(
                    q, kv[(n + 1) % RING, pl.ds(g * GK, GK), :], (((1,), (1,)), ((), ())),
                    preferred_element_type=jnp.float32)
                s_nxt[:, g * GK:(g + 1) * GK] = sg
                for j in range(TPG):
                    sj = sg[:, j * DH:(j + 1) * DH]
                    st["mx"] = sj if st["mx"] is None else jnp.maximum(st["mx"], sj)

            def do_refill():
                if refill == "ring":
                    for j in range(ND):
                        kv_pair(n + L, j)
                elif refill == "rest":
                    for j in range(ND - KOFS, ND):
                        k_tile(NT - 1, j).start(priority=0)

            for g in range(G + 1):
                if g < G:
                    do_qk(g)
                    exp_group(s_cur, m_cur, g, st)
                if g >= 1:
                    pv_group(n, g - 1, st)
                if g == G - 1:
                    do_refill()
            m_nxt[...] = jnp.broadcast_to(
                jnp.max(st["mx"], axis=-1, keepdims=True), (REP * SQ, DH))
            finish(n, st)

        def oproj(c, h, final):
            r = _ds((c % NC) * CR, CR)
            y = jnp.dot(o_scr[r, :], wo_v[_ds(h * GW, GW), :],
                        preferred_element_type=jnp.float32)
            if final:
                out_v[r, :] = (acc[r, :] + y).astype(jnp.bfloat16)
            else:
                acc[r, :] += y

        pl.loop(0, NXP)(x_pair)
        pl.loop(0, NQP)(wq_pair)
        pl.loop(0, WO_PRE)(wo_pair)
        acc[...] = jnp.zeros_like(acc)
        pltpu.make_async_copy(x_v, x_v, xsem).wait()
        pltpu.make_async_copy(wq_v, wq_v, wqsem).wait()

        @pl.loop(0, QCH)
        def _(i):
            qproj(0, _ds(i * QR, QR))
            for k in range(WO_STEP):
                wo_pair(WO_PRE + i * WO_STEP + k)

        if WO_PRE + QCH * WO_STEP < NOP:
            pl.loop(WO_PRE + QCH * WO_STEP, NOP)(wo_pair)
        for j in range(ND):
            kv_pair(0, j)

        @pl.loop(1, L)
        def _(m):
            for j in range(ND):
                kv_pair(m, j)

        k_wait(0)
        scores(0, s_a, m_a)
        pltpu.make_async_copy(wo_v, wo_v, wosem).wait()

        def body(c, carry):
            h = c // NC
            for u in range(CB):
                step(c * CB + u, u, "ring")
                if u == 1:
                    @pl.when(h < HKV - 1)
                    def _():
                        qproj(h + 1, _ds((c % NC) * CR, CR))

            @pl.when(h < HKV - 1)
            def _():
                oproj(c, h, False)

            @pl.when(h == HKV - 1)
            def _():
                oproj(c, h, True)
            return carry
        lax.fori_loop(0, NCT - 1, body, 0)

        for u in range(CB - 2):
            step((NCT - 1) * CB + u, u, "rest" if u == 0 else None)
        n = NT - 2
        k_wait(n + 1)
        scores(n + 1, s_b, m_b)
        v_wait(n)
        softmax_pv(n, s_a, m_a)
        v_wait(n + 1)
        out_bulk().start()
        softmax_pv(n + 1, s_b, m_b)
        oproj(NCT - 1, HKV - 1, True)
        out_last().start()
        out_bulk().wait()
        out_last().wait()

    anyspec = pl.BlockSpec(memory_space=pl.ANY)
    out = pl.pallas_call(
        kern,
        in_specs=[anyspec] * 5,
        out_specs=anyspec,
        out_shape=jax.ShapeDtypeStruct((M, D), jnp.bfloat16),
        scratch_shapes=[
            pltpu.VMEM((M, D), jnp.bfloat16),
            pltpu.VMEM((D, W), jnp.bfloat16),
            pltpu.VMEM((W, D), jnp.bfloat16),
            pltpu.VMEM((2, M, GW), jnp.bfloat16),
            pltpu.VMEM((M, GW), jnp.bfloat16),
            pltpu.VMEM((M, D), jnp.float32),
            pltpu.VMEM((M, D), jnp.bfloat16),
            pltpu.VMEM((2 * RING, SK, DH), jnp.bfloat16),
            pltpu.VMEM((REP * SQ, SK), jnp.float32),
            pltpu.VMEM((REP * SQ, SK), jnp.float32),
            pltpu.VMEM((REP * SQ, DH), jnp.float32),
            pltpu.VMEM((REP * SQ, DH), jnp.float32),
            pltpu.SemaphoreType.DMA((RING,)),
            pltpu.SemaphoreType.DMA((RING,)),
            pltpu.SemaphoreType.DMA(()),
            pltpu.SemaphoreType.DMA(()),
            pltpu.SemaphoreType.DMA(()),
            pltpu.SemaphoreType.DMA(()),
            pltpu.SemaphoreType.DMA(()),
        ],
        compiler_params=pltpu.CompilerParams(
            vmem_limit_bytes=64 * 1024 * 1024,
            disable_semaphore_checks=True,
            disable_bounds_checks=True,
        ),
    )(x.reshape(M, D), k_cache, v_cache, wq, wo)
    return out.reshape(B, SQ, D)
```
